```python
import os as _os
_os.environ.setdefault("JAX_PLATFORMS", "cpu")
import jax
import jax.numpy as jnp

def _softmax(x, axis=-1):
    return jax.nn.softmax(x, axis=axis)
def _gelu(x):
    return jax.nn.gelu(x, approximate=True)
def _silu(x):
    return jax.nn.silu(x)
def _sigmoid(x):
    return jax.nn.sigmoid(x)
def _layernorm(x, axis=-1, eps=1e-5):
    m = jnp.mean(x, axis=axis, keepdims=True)
    v = jnp.var(x, axis=axis, keepdims=True)
    return (x - m) / jnp.sqrt(v + eps)
def _scatter_add(tgt, idx, src, axis=0):
    return tgt.at[idx].add(src)
def _segment_sum(src, seg, n):
    return jax.ops.segment_sum(src, seg, n)
class _Rng:
    def __init__(self, key):
        self._k = key
    def _next(self):
        self._k, sub = jax.random.split(self._k)
        return sub
    def normal(self, shape):
        return jax.random.normal(self._next(), shape, dtype=jnp.bfloat16)
    def randint(self, lo, hi, shape):
        return jax.random.randint(self._next(), shape, lo, hi, dtype=jnp.int32)
    def uniform(self, shape, lo=0.0, hi=1.0):
        return jax.random.uniform(self._next(), shape, jnp.bfloat16, lo, hi)
    def permutation(self, n):
        return jax.random.permutation(self._next(), n)


kernel_name = 'concat_heads__grouped_kv_mqa__sliding_block__prompt'

def setup_inputs():
    _rng = _Rng(jax.random.key(int.from_bytes(__import__("os").urandom(4), "little")))
    _w = (lambda a: (lambda t: t.astype(jnp.bfloat16) if jnp.issubdtype(t.dtype, jnp.floating) else t)(jnp.asarray(a)))
    def _A_setup():
        B, S, D, H = 1, 2048, 576, 32
        Dh = D // H
        return {
            "x": _w((lambda *s: _rng.normal(s) * 0.05)(B, S, D)),
            "wq": _w((lambda *s: _rng.normal(s) * 1.6)(D, H * Dh)),
            "wk": _w((lambda *s: _rng.normal(s) * 1.6)(D, Dh)),
            "wv": _w((lambda *s: _rng.normal(s) * 0.1)(D, Dh)),
            "wo": _w((lambda *s: _rng.normal(s) * 0.1)(H * Dh, D)),
        }
    _A_in = _A_setup()

    def _B_setup():
        B, S, D = 1, 2048, 576
        return {
            "x": _w((lambda *s: _rng.normal(s) * 0.2)(B, S, D)),
            "wqkv": _w((lambda *s: _rng.normal(s) * 0.2)(D, 3 * D)),
            "wo": _w((lambda *s: _rng.normal(s) * 0.05)(D, D)),
        }
    _B_in = _B_setup()

    return {
        "A_x": _A_in["x"],
        "A_wq": _A_in["wq"],
        "A_wk": _A_in["wk"],
        "A_wv": _A_in["wv"],
        "A_wo": _A_in["wo"],
        "B_x": _B_in["x"],
        "B_wqkv": _B_in["wqkv"],
        "B_wo": _B_in["wo"],
    }

def reference(A_x, A_wq, A_wk, A_wv, A_wo, B_x, B_wqkv, B_wo):
    def _A_ref(x, wq, wk, wv, wo):
        B, S, D = x.shape
        H = 32
        Dh = D // H
        q = (lambda x, *d: x.transpose(*d))((x @ wq).reshape(B, S, H, Dh), 0, 2, 1, 3)
        k = x @ wk
        v = x @ wv
        scores = jnp.einsum("bhqd,bkd->bhqk", q, k) * (Dh ** -0.5)
        p = _softmax(scores, axis=-1)
        o = jnp.einsum("bhqk,bkd->bhqd", p, v)
        return (lambda x, *d: x.transpose(*d))(o, 0, 2, 1, 3).reshape(B, S, H * Dh) @ wo

    def _B_ref(x, wqkv, wo):
        B, S, D = x.shape
        H = 32; Dh = D // H; W = 256
        qkv = (lambda x, *d: x.transpose(*d))((x @ wqkv).reshape(B, S, 3, H, Dh), 2, 0, 3, 1, 4)
        q, k, v = qkv[0], qkv[1], qkv[2]
        scores = jnp.einsum("bhqd,bhkd->bhqk", q, k) * (Dh ** -0.5)
        idx = jnp.arange(S)
        mask = (idx[:, None] - idx[None, :] >= 0) & (idx[:, None] - idx[None, :] < W)
        scores = jnp.where(mask[None, None], scores, -1e9)
        p = _softmax(scores, axis=-1)
        o = jnp.einsum("bhqk,bhkd->bhqd", p, v)
        return (lambda x, *d: x.transpose(*d))(o, 0, 2, 1, 3).reshape(B, S, D) @ wo

    a = _A_ref(A_x, A_wq, A_wk, A_wv, A_wo)
    b = _B_ref(B_x, B_wqkv, B_wo)
    return jnp.concatenate([a, b], axis=-1)
```

```python
import math

import jax
import jax.numpy as jnp
from jax import lax
from jax.experimental import pallas as pl
from jax.experimental.pallas import tpu as pltpu

S, D, H, DH, WIN = 2048, 576, 32, 18, 256
T = 128
NT = S // T
TB = 512
NB = S // TB
TPB = TB // T
HG = 4
GR = HG * DH
NG = H // HG
PD = 24
LOG2E = math.log2(math.e)
QSCALE = (DH ** -0.5) * LOG2E
MASKED = -1e9 * LOG2E

F32, BF16 = jnp.float32, jnp.bfloat16


def _mm(a, b):
    return lax.dot_general(a, b, (((1,), (0,)), ((), ())), preferred_element_type=F32)


def _colmax8(s):
    return jnp.max(s.reshape(s.shape[0] // 8, 8, s.shape[1]), axis=0)


def _kernel(xa_hbm, wq_hbm, wkT_hbm, wvT_hbm, woa_hbm, xb_hbm, wqkv_hbm, wob_hbm, out_hbm,
            xa, xb, wq, wkT, wvT, woa, wob, wqkv,
            wqkvT, waT, woT,
            qb, kb, vb, ob, qa, ka, va, oa, outv,
            sa0, sa1, sa2, sa3, sb, sems, osems):
    sa = (sa0, sa1, sa2, sa3)

    def cp(i, src, dst):
        return pltpu.make_async_copy(src, dst, sems.at[i])

    c_wqkv = [cp(i, wqkv_hbm, wqkv) for i in range(1)]
    c_xb = [cp(1 + i, xb_hbm.at[:, pl.ds(i * TB, TB)], xb.at[i]) for i in range(NB)]
    c_rest = [cp(5, wq_hbm, wq), cp(6, wkT_hbm, wkT), cp(7, wvT_hbm, wvT),
              cp(8, woa_hbm, woa), cp(9, wob_hbm, wob)]
    c_xa = [cp(10 + i, xa_hbm.at[:, pl.ds(i * TB, TB)], xa.at[i]) for i in range(NB)]
    for c in [c_xb[0]] + c_wqkv + c_xb[1:] + c_xa + c_rest:
        c.start()

    c_wqkv[0].wait()
    wqkvT[...] = wqkv[...].T
    for c in c_xb:
        c.wait()

    def b_proj(i, _):
        x = xb[i]
        q = _mm(wqkvT[0:D, :], x) * QSCALE
        k = _mm(wqkvT[D:2 * D, :], x)
        v = _mm(wqkvT[2 * D:3 * D, :], x)
        for j in range(TPB):
            t = i * TPB + j
            cols = slice(j * T, (j + 1) * T)
            for g in range(NG):
                rows = slice(g * GR, (g + 1) * GR)
                qb[t, g] = q[rows, cols]
                vb[t, g] = v[rows, cols]
                kg = jnp.concatenate([k[rows, cols], jnp.zeros((T - GR, T), F32)], axis=0)
                kb[t, g] = kg.T
        return 0

    lax.fori_loop(0, NB, b_proj, 0)

    row = lax.broadcasted_iota(jnp.int32, (T, HG * T), 0)
    col = lax.broadcasted_iota(jnp.int32, (T, HG * T), 1) & (T - 1)
    causal = col >= row
    grow = lax.broadcasted_iota(jnp.int32, (GR, T), 0)
    row8 = lax.broadcasted_iota(jnp.int32, (8, T), 0)

    def b_weights(t, g):
        q = qb[t, g]
        return jnp.concatenate(
            [jnp.where((grow >= j * DH) & (grow < (j + 1) * DH), q, 0.0) for j in range(HG)], axis=1)

    def b_scores(t, g, back, w):
        s = _mm(kb[t - back, g, :, 0:GR], w)
        if back == 0:
            s = jnp.where(causal, s, MASKED)
        elif back == 2:
            s = jnp.where(causal, MASKED, s)
        sb[g, back] = s
        return _colmax8(s)

    def b_pv(t, g, back, p):
        out = []
        for j in range(HG):
            v = vb[t - back, g, 16 * j:16 * j + PD, :]
            if j == 0:
                v = jnp.concatenate([v[0:16], jnp.where(row8 == 7, 1.0, v[16:24])], axis=0)
            else:
                v = jnp.concatenate([jnp.where(row8 == 0, 1.0, v[0:8]), v[8:24]], axis=0)
            out.append(_mm(v, p[:, j * T:(j + 1) * T]))
        return out

    def b_finish(t, g, acc):
        o = []
        for j in range(HG):
            r = PD - 1 if j == 0 else 0
            o.append(acc[j] * pltpu.reciprocal(acc[j][r:r + 1, :]))
        pieces = [o[0][0:16]]
        for j in range(1, HG):
            pieces.append(jnp.where(row8 < 2 * j, o[j - 1][16:24], o[j][0:8]))
            pieces.append(o[j][8:16] if j < HG - 1 else o[j][8:24])
        ob[t, g] = jnp.concatenate(pieces, axis=0)

    def b_step(t, ms, n_old, n_new):
        new = []
        for g in range(NG):
            w = b_weights(t, g) if n_new else None
            m, acc = None, None
            for back in (2, 1, 0):
                if back < n_old:
                    p = jnp.exp2(sb[g, back] - ms[g])
                if back < n_new:
                    mm = b_scores(t, g, back, w)
                    m = mm if m is None else jnp.maximum(m, mm)
                if back < n_old:
                    r = b_pv(t - 1, g, back, p)
                    acc = r if acc is None else [a + b for a, b in zip(acc, r)]
            if n_old:
                b_finish(t - 1, g, acc)
            if n_new:
                new.append(jnp.max(m, axis=0, keepdims=True))
        return tuple(new)

    ms = b_step(0, None, 0, 1)
    ms = b_step(1, ms, 1, 2)
    ms = b_step(2, ms, 2, 3)
    ms = lax.fori_loop(3, NT, lambda t, ms: b_step(t, ms, 3, 3), ms)
    b_step(NT, ms, 3, 0)

    for c in c_xa + c_rest:
        c.wait()
    waT[0:D, :] = wq[...].T
    zpad = jnp.zeros((PD - DH, D), F32)
    waT[D:D + 2 * PD, :] = jnp.concatenate(
        [wkT[...].astype(F32), zpad, wvT[...].astype(F32), zpad], axis=0).astype(BF16)
    woT[0] = woa[...].T
    woT[1] = wob[...].T
    vrow = lax.broadcasted_iota(jnp.int32, (PD, TB), 0)

    def a_proj(i, _):
        y = _mm(waT[...], xa[i])
        q = y[0:D] * QSCALE
        k = y[D:D + PD]
        v = jnp.where(vrow == DH, 1.0, y[D + PD:D + 2 * PD])
        for j in range(TPB):
            t = i * TPB + j
            cols = slice(j * T, (j + 1) * T)
            for g in range(NG):
                qa[t, g] = q[g * GR:(g + 1) * GR, cols]
            ka[t] = jnp.concatenate([k[:, cols], jnp.zeros((T - PD, T), F32)], axis=0).T
            va[t] = v[:, cols]
        return 0

    lax.fori_loop(0, NB, a_proj, 0)

    def a_step(it, ms, old, new):
        if new:
            blk, g = it // NG, it % NG
            qg = jnp.concatenate([qa[blk * TPB + i, g] for i in range(TPB)], axis=1)
        outs, mnew = [], []
        for j in range(HG):
            if new:
                w = jnp.concatenate([qg[j * DH:(j + 1) * DH], jnp.zeros((PD - DH, TB), F32)], axis=0)
            m, acc = None, None
            for c in range(NT):
                if old:
                    p = jnp.exp2(sa[j][c] - ms[j])
                if new:
                    s = _mm(ka[c, :, 0:PD], w)
                    sa[j][c] = s
                    mm = _colmax8(s)
                    m = mm if m is None else jnp.maximum(m, mm)
                if old:
                    r = _mm(va[c], p)
                    acc = r if acc is None else acc + r
            if old:
                outs.append((acc * pltpu.reciprocal(acc[DH:DH + 1, :]))[0:DH])
            if new:
                mnew.append(jnp.max(m, axis=0, keepdims=True))
        if old:
            blk, g = (it - 1) // NG, (it - 1) % NG
            o = jnp.concatenate(outs, axis=0)
            for i in range(TPB):
                oa[blk * TPB + i, g] = o[:, i * T:(i + 1) * T]
        return tuple(mnew)

    ms = a_step(0, None, False, True)
    ms = lax.fori_loop(1, NB * NG, lambda it, ms: a_step(it, ms, True, True), ms)
    a_step(NB * NG, ms, True, False)

    def out_copy(i):
        return pltpu.make_async_copy(outv.at[i], out_hbm.at[pl.ds(i * TB, TB), :], osems.at[i])

    def out_proj(i, _):
        ys = []
        for n, o in enumerate((oa, ob)):
            ot = jnp.concatenate([o[i * TPB + j].reshape(D, T) for j in range(TPB)], axis=1)
            ys.append(_mm(woT[n], ot.astype(BF16)))
        outv[i] = jnp.concatenate(ys, axis=0).astype(BF16).T
        out_copy(i).start()
        return 0

    lax.fori_loop(0, NB, out_proj, 0)
    for i in range(NB):
        out_copy(i).wait()


@jax.jit
def pallas_concat_heads__grouped_kv_mqa__sliding_block__prompt_kernel(A_x, A_wq, A_wk, A_wv, A_wo, B_x, B_wqkv, B_wo):
    hbm = pl.BlockSpec(memory_space=pltpu.HBM)
    vm = pltpu.VMEM
    act = vm((NT, NG, GR, T), F32)
    out = pl.pallas_call(
        _kernel,
        out_shape=jax.ShapeDtypeStruct((S, 2 * D), BF16),
        in_specs=[hbm] * 8,
        out_specs=hbm,
        scratch_shapes=[
            vm((NB, D, TB), BF16), vm((NB, D, TB), BF16),
            vm((D, D), BF16), vm((DH, D), BF16), vm((DH, D), BF16),
            vm((D, D), BF16), vm((D, D), BF16), vm((D, 3 * D), BF16),
            vm((3 * D, D), BF16), vm((D + 2 * PD, D), BF16), vm((2, D, D), BF16),
            act, vm((NT, NG, T, T), F32), act, act,
            act, vm((NT, T, T), F32), vm((NT, PD, T), F32), act,
            vm((NB, TB, 2 * D), BF16),
            vm((NT, T, TB), F32), vm((NT, T, TB), F32), vm((NT, T, TB), F32), vm((NT, T, TB), F32),
            vm((NG, 3, T, HG * T), F32),
            pltpu.SemaphoreType.DMA((14,)), pltpu.SemaphoreType.DMA((NB,)),
        ],
        compiler_params=pltpu.CompilerParams(vmem_limit_bytes=110 * 2**20),
        name="attn2",
    )(A_x[0].T, A_wq, A_wk.T, A_wv.T, A_wo, B_x[0].T, B_wqkv, B_wo)
    return out[None]
```

```python
import functools
import math

import jax
import jax.numpy as jnp
from jax import lax
from jax.experimental import pallas as pl
from jax.experimental.pallas import tpu as pltpu

S, D, H, WINDOW = 2048, 576, 32, 256
DH = D // H
T = 128
NT = S // T
TB = 512
NB = S // TB
TPB = TB // T
HG = 4
GR = HG * DH
NG = H // HG
PD = 24
RG = T // 8
SUB = T // HG
NR = WINDOW // SUB + 1
SPLIT = 5 * T
A_UNITS = 16
B_TILES = 2

LOG2E = math.log2(math.e)
SCALE = DH ** -0.5 * LOG2E
MASKED = -1e9 * LOG2E
DENOMINATOR_MIN = 2.0 ** -40
SUM_MAX = 2.0 ** 120

_THREE = ((3, 2, 1), (7, 6, 5), (11, 10, 9), (15, 14, 13))
VPU_SLOTS = (
    _THREE, ((4, 3, 10), (6, 5, 8), (10, 9, 8), (14, 13, 8)), _THREE, _THREE,
    _THREE, ((2, 1, 8), (6, 5, 8), (10, 9, 8), (14, 13, 8)), _THREE,
    ((3, 2, 1), (11, 10, 9), (7, 6, 5), (15, 14, 13)),
    ((3, 2, 1), (7, 6, 5), (10, 9, 8), (15, 14, 13)),
    ((2, 1, 8), (6, 5, 8), (10, 9, 8), (14, 13, 8)), _THREE,
    ((3, 2, 1), (7, 6, 5), (11, 8, 9), (15, 14, 13)),
    ((3, 2, 1), (7, 6, 5), (10, 11, 9), (15, 14, 13)),
    ((2, 1, 8), (7, 6, 9), (10, 9, 8), (14, 13, 8)), _THREE,
    ((2, 1), (6, 5), (12, 11), (14, 13)),
)
EARLY = (1, 5, 9, 13)
EARLY_CUTS = (0, 40, 84, 128)
AHEAD = (0, 2, 3, 3, 3, 3, 3, 4, 3, 3, 4, 3, 3, 3, 3, 3, 0)

F32, BF16, I32 = jnp.float32, jnp.bfloat16, jnp.int32


def _mm(a, b):
    return lax.dot_general(a, b, (((1,), (0,)), ((), ())), preferred_element_type=F32)


def _iota(shape, axis):
    return lax.broadcasted_iota(I32, shape, axis)


def _aligned(i, n):
    return i if isinstance(i, int) else pl.multiple_of(i, n)


def _tile(i):
    return slice(i * T, (i + 1) * T)


def _pad_rows(x, rows):
    return jnp.concatenate([x, jnp.zeros((rows - x.shape[0], x.shape[1]), F32)], axis=0)


def _fold8(op, x):
    return op(x.reshape(x.shape[0] // 8, 8, x.shape[1]), axis=0)


def _inverse(x):
    y = pltpu.reciprocal(x, approx=True)
    return y * (2.0 - x * y)


def _put_rows(ref, lo, x, cols=slice(None)):
    ref[lo // 2:(lo + x.shape[0]) // 2, cols] = pltpu.bitcast(x, I32)


def _rows(ref, lo, hi, cols=slice(None)):
    return pltpu.bitcast(ref[lo // 2:hi // 2, cols], BF16)


def _key_order(slots):
    mxu = iter(range(RG - len(slots) - 1, -1, -1))
    return [RG - len(slots) + slots.index(s) if s in slots else next(mxu) for s in range(RG)]


def _query_rows(qa, u, i):
    return [jnp.broadcast_to(qa[u, d:d + 1, _tile(i)], (8, T)) for d in range(DH)]


def _vpu_scores(keys, q):
    s = keys[0] * q[0]
    for d in range(1, DH):
        s = s + keys[d] * q[d]
    return s


def _a_pv(vperm, c, p):
    return jnp.concatenate([_mm(vperm[c, :, _tile(i)], p[i]) for i in range(TPB)], axis=1)


def _a_keep(oa, slot, acc, low, total):
    oa[slot] = acc
    for i in range(TPB):
        low = jnp.minimum(low, acc[16:PD, _tile(i)])
        total = total + _fold8(jnp.sum, jnp.abs(acc[:, _tile(i)]))
    return low, total


def _a_step(qa, ka, kcol, vperm, early, plast, oa, step, carry):
    acc, low, total = carry
    p, spill = [plast[i] for i in range(TPB)], None
    for j in range(A_UNITS):
        u = step * A_UNITS + j
        q = [jnp.concatenate(x, axis=1) for x in zip(*(_query_rows(qa, u, i) for i in range(TPB)))]
        w = qa[u]
        for c in range(NT):
            nv = len(VPU_SLOTS[c][0])
            done, more = 8 * AHEAD[c], 8 * AHEAD[c + 1]
            keys = ka[c, done:T - 8 * nv, 0:PD]
            if more:
                keys = jnp.concatenate([keys, ka[c + 1, 0:more, 0:PD]], axis=0)
            s = _mm(keys, w)
            if done:
                s = jnp.concatenate([spill, s], axis=0)
            spill = s[s.shape[0] - more:] if more else None
            e = [jnp.exp2(s[0:T - 8 * nv])]
            n = nv - (c in EARLY)
            keys = [jnp.concatenate([kcol[c, d, 0:n]] * TPB, axis=-1) for d in range(DH)]
            e.append(jnp.exp2(_vpu_scores(keys, q)).reshape(8 * n, TB))
            if c in EARLY:
                e.append(early[EARLY.index(c), u])
            e = jnp.concatenate(e, axis=0)
            r = _a_pv(vperm, (c - 1) % NT, p)
            acc = r if c == 1 else acc + r
            if c == 0:
                low, total = _a_keep(oa, u, acc, low, total)
            e = [e[r:r + 8] for r in range(0, T, 8)]
            p = [jnp.concatenate([e[r] for r in _key_order(VPU_SLOTS[c][i])], axis=0)[:, _tile(i)]
                 for i in range(TPB)]
    for i in range(TPB):
        plast[i] = p[i]
    return acc, low, total


def _kernel(xa_hbm, wq_hbm, wk_hbm, wv_hbm, woa_hbm, xb_hbm, wqkv_hbm, wob_hbm, out_hbm,
            qa, ka, kcol, kearly, vperm, va, oa, early, plast,
            xa, xb, wq, wkv, woa, wob, wqkv, wqkv_t, wa_t, wo_t,
            qb, kb, vb, ob, sb, qmask, cap, yb, out, sfull,
            in_sems, xb_sems, out_sems):
    fetched, stored = [], []

    def fetch(src, dst):
        fetched.append(pltpu.make_async_copy(src, dst, in_sems.at[len(fetched)]))
        fetched[-1].start()
        return [fetched[-1]]

    def store(i, lo, hi):
        stored.append(pltpu.make_async_copy(
            out.at[i, :, pl.ds(lo, hi - lo)], out_hbm.at[pl.ds(i * TB, TB), pl.ds(lo, hi - lo)],
            out_sems.at[len(stored)]))
        stored[-1].start()
        return [stored[-1]]

    def xb_copy(i):
        return pltpu.make_async_copy(
            xb_hbm.at[:, pl.ds(_aligned(i * TB, TB), TB)], xb.at[i], xb_sems.at[i])

    def wait(copies):
        for c in copies:
            c.wait()

    pieces = (slice(0, T), slice(T, 3 * T), slice(3 * T, D))
    wait_first = [fetch(wq_hbm.at[k], wq.at[k]) + fetch(xa_hbm.at[k, 0:TB], xa.at[0, k]) for k in pieces]
    wait_first[-1] += fetch(wk_hbm, wkv.at[0]) + fetch(wv_hbm, wkv.at[1])
    wait_xa = [fetch(xa_hbm.at[:, pl.ds(i * TB, TB)], xa.at[i]) for i in range(1, NB)]
    columns = (slice(0, 6 * T), slice(6 * T, 3 * D))
    wait_wqkv = [fetch(wqkv_hbm.at[:, c], wqkv.at[:, c]) for c in columns]
    for i in range(NB):
        xb_copy(i).start()
    wait_wo = fetch(woa_hbm, woa) + fetch(wob_hbm, wob)

    head = sum((_iota((GR, T), 0) >= h * DH).astype(I32) for h in range(1, HG))
    variant = ((_iota((GR, T), 1) >> 5) - head) & (HG - 1)
    for v in range(HG):
        qmask[v] = jnp.where(variant == v, -1, 0)
    causal = (_iota((SUB, T), 1) & (SUB - 1)) >= _iota((SUB, T), 0)
    cap[0] = jnp.where(causal, MASKED, jnp.inf)
    cap[1] = jnp.where(causal, jnp.inf, MASKED)
    block = _iota((SUB, T), 1) >> 5
    odd, upper = (block & 1) == 1, block >= 2
    row8 = _iota((8, T), 0)

    def zeros(rows):
        return jnp.concatenate([(qmask[0, 0:8] & qmask[1, 0:8]).astype(F32)] * (rows // 8), axis=0)

    def a_queries(i, q, h0=0):
        for j in range(TPB):
            for h in range(q.shape[0] // DH):
                qa[i * H + h0 + h, :, _tile(j)] = _pad_rows(q[h * DH:(h + 1) * DH, _tile(j)], PD)

    def a_keys(i, kv, centre):
        k = kv[0:PD] * SCALE - centre
        for j in range(TPB):
            t = i * TPB + j
            kt = _pad_rows(k[:, _tile(j)], T).T
            ka[t] = kt
            va[t] = jnp.where(_iota((PD, T), 0) == DH, 1.0, kv[PD:2 * PD, _tile(j)])
            if t in EARLY:
                for d in range(DH):
                    kearly[EARLY.index(t), d] = jnp.broadcast_to(kt[T - 8:T, d:d + 1], (8, T))

    wait(wait_first[0])
    for n, k in enumerate(pieces):
        _put_rows(wa_t, 0, wq[k, :].T, k)
        if n + 1 < len(pieces):
            x = [_mm(_rows(wa_t, 0, D - T, k), xa[0, k, :])]
            wait(wait_first[n + 1])
            x = jnp.concatenate(x + [_mm(_rows(wa_t, D - T, D, k), xa[0, k, :])], axis=0)
        else:
            x = _mm(_rows(wa_t, 0, D, k), xa[0, k, :])
        q = q + x if n else x
    a_queries(0, q)
    _put_rows(wa_t, D, jnp.concatenate(
        [_pad_rows(wkv[n].astype(F32), PD) for n in range(2)], axis=0).astype(BF16))
    for i in range(1, NB):
        wait(wait_xa[i - 1] + (wait_wqkv[0] if i == NB - 1 else []))
        if i == 1:
            kv0 = _mm(_rows(wa_t, D, D + 2 * PD), xa[0])
            centre = jnp.sum(kv0[0:PD], axis=1, keepdims=True) * (SCALE / TB)
        kv = _mm(_rows(wa_t, D, D + 2 * PD), xa[i])
        if i < NB - 1:
            a_queries(i, _mm(_rows(wa_t, 0, D // 2), xa[i]))
            if i == 1:
                a_keys(0, kv0, centre)
            a_keys(i, kv, centre)
        else:
            a_keys(i, kv, centre)
            _put_rows(wqkv_t, columns[0].start, wqkv[:, columns[0]].T)
            a_queries(i, _mm(_rows(wa_t, 0, D // 2), xa[i]))
            wait(wait_wqkv[1])
            _put_rows(wqkv_t, columns[1].start, wqkv[:, columns[1]].T)
        a_queries(i, _mm(_rows(wa_t, D // 2, D), xa[i]), H // 2)

    def join_heads(o):
        rows = [o[0][0:16]]
        for h in range(1, HG):
            rows.append(jnp.where(row8 < 2 * h, o[h - 1][16:24], o[h][0:8]))
            rows.append(o[h][8:16] if h < HG - 1 else o[h][8:24])
        return jnp.concatenate(rows, axis=0)

    xb_copy(0).wait()

    @pl.loop(0, NB)
    def _(i):
        for part in range(3):
            keys = [kearly[i, d] for d in range(DH)]
            for u in range(EARLY_CUTS[part], EARLY_CUTS[part + 1]):
                for j in range(TPB):
                    early[i, u, :, _tile(j)] = jnp.exp2(_vpu_scores(keys, _query_rows(qa, u, j)))
            y = _mm(_rows(wqkv_t, part * D, (part + 1) * D), xb[i])
            for j in range(TPB):
                t = i * TPB + j
                for g in range(NG):
                    x = y[g * GR:(g + 1) * GR, _tile(j)]
                    if part == 0:
                        x = x * SCALE
                        qb[t, g] = join_heads(
                            [pltpu.roll(x[16 * h:16 * h + PD], h * SUB, 1) if h else x[0:PD]
                             for h in range(HG)])
                    elif part == 1:
                        kb[g, pl.ds(pl.multiple_of(t * T, T), T), :] = _pad_rows(x, T).T
                    else:
                        vb[t, g, 0] = jnp.concatenate(
                            [x[0:16], jnp.where(row8 == 7, 1.0, x[16:24])], axis=0)
                        for h in range(1, HG):
                            vb[t, g, h] = jnp.concatenate(
                                [jnp.where(row8 == 0, 1.0, x[16 * h:16 * h + 8]), x[16 * h + 8:16 * h + PD]],
                                axis=0)
        pl.when(i + 1 < NB)(lambda: xb_copy(jnp.minimum(i + 1, NB - 1)).wait())

    offset = _iota((8, T), 1) - row8
    for slots in dict.fromkeys(VPU_SLOTS):
        tiles = [c for c in range(NT) if VPU_SLOTS[c] == slots]
        moves = [jnp.concatenate([jnp.where(offset == 8 * order.index(r), 1.0, 0.0) for r in range(RG)], axis=0)
                 for order in map(_key_order, slots)]
        moved = _mm(jnp.concatenate([va[c] for c in tiles], axis=0), jnp.concatenate(moves, axis=1))
        for n, c in enumerate(tiles):
            vperm[c] = moved[n * PD:(n + 1) * PD]

    def pick(mask, a, b):
        if a is None and b is None:
            return None
        return jnp.where(mask, 0.0 if a is None else a, 0.0 if b is None else b)

    def first_key(t):
        return max(0, (WINDOW - t * T) // SUB) if isinstance(t, int) else 0

    def b_probs(n, m, kt):
        heads = [[] for _ in range(HG)]
        for b in range(kt * HG, (kt + 1) * HG):
            y = [jnp.exp2(sb[n, v, (b - v) * SUB:(b - v + 1) * SUB, :] - m[v]) if 0 <= b - v < NR else None
                 for v in range(HG)]
            z = [pick(odd, y[(v + 1) % HG], y[v]) for v in range(HG)]
            for h in range(HG):
                heads[h].append(pick(upper, z[(2 - h) % HG], z[(-h) % HG]))
        return [jnp.concatenate(x, axis=0) for x in heads]

    def b_scores(t, g, v, w, lo, hi):
        start = _aligned(t * T + (v + lo) * SUB - WINDOW, SUB)
        s = _mm(kb[g, pl.ds(start, (hi - lo) * SUB), 0:GR], w)
        s = [s[r * SUB:(r + 1) * SUB] for r in range(hi - lo)]
        if lo == 0:
            s[0] = jnp.minimum(s[0], cap[0])
        if hi == NR:
            s[-1] = jnp.minimum(s[-1], cap[1])
        return jnp.concatenate(s, axis=0)

    def b_step(t0, maxima, new, filler=()):
        weights, m = {}, {}

        def scores(n, part):
            t, g = t0 + n // NG, n % NG
            if n not in weights:
                q = pltpu.bitcast(qb[t, g], I32)
                weights[n] = [pltpu.bitcast(q & qmask[v], F32) for v in range(HG)]
            for v in range(HG):
                lo, hi = max(3 * part, first_key(t) - v), 3 * part + 3
                if lo < hi:
                    s = b_scores(t, g, v, weights[n][v], lo, hi)
                    sb[n, v, lo * SUB:hi * SUB, :] = s
                    s = _fold8(jnp.max, s)
                    m[n, v] = jnp.maximum(m[n, v], s) if (n, v) in m else s

        units = range(B_TILES * NG)
        todo = [functools.partial(scores, n, part) for n in units for part in range(3) if new]
        todo += list(filler)
        for n in units if maxima is not None else ():
            t, g = t0 - B_TILES + n // NG, n % NG
            acc = [zeros(PD)] * HG
            for kt in range(3):
                if kt * HG >= first_key(t):
                    p = b_probs(n, maxima[n], kt)
                    acc = [acc[h] + _mm(vb[t - 2 + kt, g, h], p[h]) for h in range(HG)]
                if todo and (n, kt) != (0, 0):
                    todo.pop(0)()
            o = [acc[h] * _inverse(acc[h][0:1, :] if h else acc[h][PD - 1:PD, :]) for h in range(HG)]
            ob[t, g] = join_heads([pltpu.roll(o[h], T - h * SUB, 1) if h else o[h] for h in range(HG)])
        for work in todo:
            work()
        if new:
            return tuple(tuple(jnp.max(m[n, v], axis=0, keepdims=True) for v in range(HG)) for n in units)

    maxima = b_step(0, None, True)
    wait(wait_wo)
    maxima = b_step(B_TILES, maxima, True)
    _put_rows(wo_t, D, wob[...].T)
    maxima = lax.fori_loop(2, NT // B_TILES, lambda i, m: b_step(i * B_TILES, m, True), maxima)

    def b_heads(i):
        return jnp.concatenate([ob[i * TPB + j].reshape(D, T) for j in range(TPB)], axis=1)

    rows, sums = 96, {}

    def b_project(i, lo, k):
        ks = slice(k * T, min((k + 1) * T, D))
        y = _mm(_rows(wo_t, D + lo, D + lo + rows, ks), b_heads(i)[ks])
        sums[i, lo] = y + (sums[i, lo] if k else jnp.concatenate([zeros(rows)] * TPB, axis=1))

    b_step(NT, maxima, False, [functools.partial(b_project, i, lo, k)
                               for i in range(2) for lo in range(0, D, rows) for k in range(pl.cdiv(D, T))])
    for i in range(NB):
        if i < 2:
            y = jnp.concatenate([sums[i, lo] for lo in range(0, D, rows)], axis=0)
        else:
            y = _mm(_rows(wo_t, D, 2 * D), b_heads(i).astype(BF16))
        y = y.astype(BF16)
        yb[i] = y[0:SPLIT - D]
        out[i, :, SPLIT:2 * D] = y[SPLIT - D:D].T
    _put_rows(wo_t, 0, woa[...].T)
    for d in range(DH):
        for t in range(NT):
            lo, hi = T - 8 * len(VPU_SLOTS[t][0]), T - 8 * (t in EARLY)
            kcol[t, d, 0:(hi - lo) // 8] = jnp.broadcast_to(
                ka[t, lo:hi, :][:, d:d + 1], (hi - lo, T)).reshape(-1, 8, T)
    pending = [c for i in range(NB) for c in store(i, SPLIT, 2 * D)]

    plast[...] = jnp.zeros(plast.shape, F32)
    acc, low, total = lax.fori_loop(
        0, NB * H // A_UNITS, functools.partial(_a_step, qa, ka, kcol, vperm, early, plast, oa),
        (jnp.ones((PD, TB), F32), jnp.ones((8, T), F32), jnp.zeros((8, T), F32)))

    def a_heads(i):
        o = [oa[i * H + h + 1] for h in range(H)]
        return jnp.concatenate([(x * _inverse(x[DH:DH + 1, :]))[0:DH] for x in o], axis=0).astype(BF16)

    for i in range(NB):
        x = a_heads(i)
        for lo, hi in ((0, SPLIT),) if i < NB - 1 else ((0, 3 * T), (3 * T, SPLIT)):
            y = _mm(_rows(wo_t, lo, min(hi, D)), x).astype(BF16)
            if i == 1:
                acc = acc + _a_pv(vperm, NT - 1, [plast[j] for j in range(TPB)])
                low, total = _a_keep(oa, NB * H, acc, low, total)
                safe = (total <= SUM_MAX) & ((row8 != DH - 16) | (low >= DENOMINATOR_MIN))
                unsafe = jnp.max(jnp.where(safe, 0.0, 1.0))
            if i >= 2:
                pending.pop(0).wait()
            out[i, :, lo:hi] = (jnp.concatenate([y, yb[i]], axis=0) if hi > D else y).T
            pending += store(i, lo, hi)
    wait(pending)

    @pl.when(unsafe > 0.0)
    def _():
        for i in range(NB):
            a_keys(i, _mm(_rows(wa_t, D, D + 2 * PD), xa[i]), 0.0)

        @pl.loop(0, NB * H)
        def _(u):
            w = qa[u]

            def scores(c, m):
                s = _mm(ka[c, :, 0:PD], w)
                sfull[c] = s
                return jnp.maximum(m, _fold8(jnp.max, s))

            m = lax.fori_loop(0, NT, scores, jnp.full((8, TB), -jnp.inf, F32))
            m = jnp.max(m, axis=0, keepdims=True)
            oa[u + 1] = lax.fori_loop(
                0, NT, lambda c, o: o + _mm(va[c], jnp.exp2(sfull[c] - m)), jnp.zeros((PD, TB), F32))

        @pl.loop(0, NB)
        def _(i):
            y = _mm(_rows(wo_t, 0, D), a_heads(i)).astype(BF16)
            out[i, :, 0:SPLIT] = jnp.concatenate([y, yb[i]], axis=0).T
            c = pltpu.make_async_copy(
                out.at[i], out_hbm.at[pl.ds(pl.multiple_of(i * TB, TB), TB)], out_sems.at[0])
            c.start()
            c.wait()


@jax.jit
def pallas_concat_heads__grouped_kv_mqa__sliding_block__prompt_kernel(
    A_x: jax.Array,
    A_wq: jax.Array,
    A_wk: jax.Array,
    A_wv: jax.Array,
    A_wo: jax.Array,
    B_x: jax.Array,
    B_wqkv: jax.Array,
    B_wo: jax.Array,
):
    hbm = pl.BlockSpec(memory_space=pltpu.HBM)
    vmem = pltpu.VMEM
    out = pl.pallas_call(
        _kernel,
        out_shape=jax.ShapeDtypeStruct((S, 2 * D), BF16),
        in_specs=[hbm] * 8,
        out_specs=hbm,
        scratch_shapes=[
            vmem((NB * H, PD, TB), F32),
            vmem((NT, T, T), F32),
            vmem((NT, DH, 3, 8, T), F32),
            vmem((NB, DH + 2, 8, T), F32),
            vmem((NT, PD, TB), F32),
            vmem((NT, PD, T), F32),
            vmem((NB * H + 1, PD, TB), F32),
            vmem((NB, NB * H, 8, TB), F32),
            vmem((TPB, T, T), F32),
            vmem((NB, D, TB), BF16),
            vmem((NB, D, TB), BF16),
            vmem((D, D), BF16),
            vmem((8, DH, D), BF16),
            vmem((D, D), BF16),
            vmem((D, D), BF16),
            vmem((D, 3 * D), BF16),
            vmem((3 * D // 2, D), I32),
            vmem((SPLIT // 2, D), I32),
            vmem((D, D), I32),
            vmem((NT, NG, GR, T), F32),
            vmem((NG, S, T), F32),
            vmem((NT, NG, HG, PD, T), F32),
            vmem((NT, NG, GR, T), F32),
            vmem((B_TILES * NG, HG, NR * SUB, T), F32),
            vmem((HG, GR, T), I32),
            vmem((2, SUB, T), F32),
            vmem((NB, SPLIT - D, TB), BF16),
            vmem((NB, TB, 2 * D), BF16),
            vmem((NT, T, TB), F32),
            pltpu.SemaphoreType.DMA((15,)),
            pltpu.SemaphoreType.DMA((NB,)),
            pltpu.SemaphoreType.DMA((2 * NB + 1,)),
        ],
        compiler_params=pltpu.CompilerParams(vmem_limit_bytes=120 * 2**20),
        name="attn2",
    )(A_x[0].T, A_wq, A_wk.T, A_wv.T, A_wo, B_x[0].T, B_wqkv, B_wo)
    return out[None]
```
